```python
import os as _os
_os.environ.setdefault("JAX_PLATFORMS", "cpu")
import jax
import jax.numpy as jnp

def _softmax(x, axis=-1):
    return jax.nn.softmax(x, axis=axis)
def _gelu(x):
    return jax.nn.gelu(x, approximate=True)
def _silu(x):
    return jax.nn.silu(x)
def _sigmoid(x):
    return jax.nn.sigmoid(x)
def _layernorm(x, axis=-1, eps=1e-5):
    m = jnp.mean(x, axis=axis, keepdims=True)
    v = jnp.var(x, axis=axis, keepdims=True)
    return (x - m) / jnp.sqrt(v + eps)
def _scatter_add(tgt, idx, src, axis=0):
    return tgt.at[idx].add(src)
def _segment_sum(src, seg, n):
    return jax.ops.segment_sum(src, seg, n)
class _Rng:
    def __init__(self, key):
        self._k = key
    def _next(self):
        self._k, sub = jax.random.split(self._k)
        return sub
    def normal(self, shape):
        return jax.random.normal(self._next(), shape, dtype=jnp.bfloat16)
    def randint(self, lo, hi, shape):
        return jax.random.randint(self._next(), shape, lo, hi, dtype=jnp.int32)
    def uniform(self, shape, lo=0.0, hi=1.0):
        return jax.random.uniform(self._next(), shape, jnp.bfloat16, lo, hi)
    def permutation(self, n):
        return jax.random.permutation(self._next(), n)


kernel_name = 'concat_heads__ssm_conv_s4__linear_attn_block__prompt'

def setup_inputs():
    _rng = _Rng(jax.random.key(int.from_bytes(__import__("os").urandom(4), "little")))
    _w = (lambda a: (lambda t: t.astype(jnp.bfloat16) if jnp.issubdtype(t.dtype, jnp.floating) else t)(jnp.asarray(a)))
    def _A_setup():
        B, L, D, N = 1, 2048, 512, 128
        A_re = -jnp.exp((lambda *s: _rng.normal(s) * 0.1)(D, N))
        A_im = jnp.pi * (lambda *s: _rng.normal(s) * 0.1)(D, N)
        B_re = (lambda *s: _rng.normal(s) * 0.1)(D, N)
        B_im = (lambda *s: _rng.normal(s) * 0.1)(D, N)
        C_re = (lambda *s: _rng.normal(s) * 0.1)(D, N)
        C_im = (lambda *s: _rng.normal(s) * 0.1)(D, N)
        log_dt = (lambda *s: _rng.normal(s) * 0.1)(D) * 0.5 - 4.0
        Dskip = (lambda *s: _rng.normal(s) * 0.05)(D)
        return {
            "u": _w((lambda *s: _rng.normal(s) * 0.05)(B, L, D)),
            "A_re": _w(A_re),
            "A_im": _w(A_im),
            "B_re": _w(B_re),
            "B_im": _w(B_im),
            "C_re": _w(C_re),
            "C_im": _w(C_im),
            "log_dt": _w(log_dt),
            "Dskip": _w(Dskip),
        }
    _A_in = _A_setup()

    def _B_setup():
        B, S, D = 1, 2048, 512
        return {
            "x": _w((lambda *s: _rng.normal(s) * 0.05)(B, S, D)),
            "wqkv": _w((lambda *s: _rng.normal(s) * 0.4)(D, 3 * D)),
            "wo": _w((lambda *s: _rng.normal(s) * 0.05)(D, D)),
        }
    _B_in = _B_setup()

    return {
        "A_u": _A_in["u"],
        "A_A_re": _A_in["A_re"],
        "A_A_im": _A_in["A_im"],
        "A_B_re": _A_in["B_re"],
        "A_B_im": _A_in["B_im"],
        "A_C_re": _A_in["C_re"],
        "A_C_im": _A_in["C_im"],
        "A_log_dt": _A_in["log_dt"],
        "A_Dskip": _A_in["Dskip"],
        "B_x": _B_in["x"],
        "B_wqkv": _B_in["wqkv"],
        "B_wo": _B_in["wo"],
    }

def reference(A_u, A_A_re, A_A_im, A_B_re, A_B_im, A_C_re, A_C_im, A_log_dt, A_Dskip, B_x, B_wqkv, B_wo):
    def _A_ref(u, A_re, A_im, B_re, B_im, C_re, C_im, log_dt, Dskip):
        Bsz, L, D = u.shape
        dt = jnp.exp(log_dt)[:, None]
        A = A_re + 1j * A_im
        Bc = B_re + 1j * B_im
        Cc = C_re + 1j * C_im
        logdA = dt * A
        dB = dt * Bc
        l = (lambda x, dt: x.astype(dt))(jnp.arange(L), A_re.dtype)
        P = jnp.exp(logdA[:, :, None] * l[None, None, :])
        K = jnp.einsum("dn,dnl,dn->dl", Cc, P, dB).real
        L2 = 2 * L
        Kp = jnp.pad(K, ((0, 0), (0, L)))
        up = (lambda x, *d: x.transpose(*d))(u, 0, 2, 1)
        up = jnp.pad(up, ((0, 0), (0, 0), (0, L)))
        Kf = (lambda x, axes=(-2,-1): jnp.fft.rfft2(x.astype(jnp.float32), axes=axes))(Kp[:, None, :], axes=(-2, -1))
        Uf = (lambda x, axes=(-2,-1): jnp.fft.rfft2(x.astype(jnp.float32), axes=axes))(up[:, :, None, :], axes=(-2, -1))
        Yf = Uf * Kf[None, :, :, :]
        y = (lambda x, s, axes=(-2,-1): jnp.fft.irfft2(x, s=s, axes=axes).astype(jnp.bfloat16))(Yf, (1, L2), axes=(-2, -1))[:, :, 0, :L]
        y = (lambda x, *d: x.transpose(*d))(y, 0, 2, 1) + u * Dskip[None, None, :]
        return y

    def _B_ref(x, wqkv, wo):
        B, S, D = x.shape
        H = 32; Dh = D // H
        qkv = (lambda x, *d: x.transpose(*d))((x @ wqkv).reshape(B, S, 3, H, Dh), 2, 0, 3, 1, 4)
        q, k, v = qkv[0], qkv[1], qkv[2]
        phi = lambda t: jnp.where(t > 0, t + 1, jnp.exp(t)) + 1e-6
        pq, pk = phi(q), phi(k)
        kv = jnp.einsum("bhsd,bhse->bhde", pk, v)
        z = jnp.einsum("bhsd->bhd", pk)
        num = jnp.einsum("bhqd,bhde->bhqe", pq, kv)
        den = jnp.einsum("bhqd,bhd->bhq", pq, z)[..., None] + 1e-6
        o = num / den
        return (lambda x, *d: x.transpose(*d))(o, 0, 2, 1, 3).reshape(B, S, D) @ wo

    a = _A_ref(A_u, A_A_re, A_A_im, A_B_re, A_B_im, A_C_re, A_C_im, A_log_dt, A_Dskip)
    b = _B_ref(B_x, B_wqkv, B_wo)
    return jnp.concatenate([a, b], axis=-1)
```

```python
import numpy as np
import jax
import jax.numpy as jnp
from jax import lax
import jax.experimental.pallas as pl
import jax.experimental.pallas.tpu as pltpu

L, D, N, T, NB = 2048, 512, 128, 128, 16
f32, bf16 = jnp.float32, jnp.bfloat16
PW = {1: 0, 2: 1, 4: 2, 8: 3, 16: 4, 32: 5, 64: 6, 256: 7, 512: 8, 1024: 9, 2048: 10, 252: 11}
CI = 12


def _constants():
    k = np.arange(T) + 0.5
    ang = 2 * np.pi * np.outer(k, np.arange(T)) / (2 * T)
    F = np.concatenate([np.cos(ang), -np.sin(ang)], 0)
    ang2 = 2 * np.pi * np.outer(np.arange(T) + T, k) / (2 * T)
    Fi = np.concatenate([np.cos(ang2), -np.sin(ang2)], 1) / T
    off = [[0, 4, 256, 512, 1024, 2048], [1, 5, 258, 516, 1280, -1],
           [2, 6, 260, 768, 1536, -1], [3, 7, 262, 772, 1792, -1]]
    slot = {}
    for c in range(4):
        for q in range(6):
            for b in range(32):
                if off[c][q] >= 0:
                    slot.setdefault(off[c][q] + 8 * b, (q, c * 32 + b))
    lr = np.arange(L).astype(np.float32).view(np.uint32)
    lr = ((lr + 0x7FFF + ((lr >> 16) & 1)) & 0xFFFF0000).astype(np.uint32).view(np.float32).astype(int)
    units = {}
    for j in range(L):
        q, ln = slot[lr[j]]
        g = units.setdefault((q, j // T), np.zeros((2 * T, T)))
        g[:, ln] += F[:, j % T]
    keys = sorted(units)
    G = np.stack([units[x] for x in keys])
    ones = np.kron(np.eye(8), np.ones((16, 16)))
    cast = lambda a: np.asarray(a, np.float32).astype(jnp.bfloat16)
    return cast(F), cast(Fi), cast(G), keys, cast(ones)


_F, _FI, _G, _KEYS, _ONES = _constants()


def _cmul(a, b):
    return (a[0] * b[0] - a[1] * b[1], a[0] * b[1] + a[1] * b[0])


def _kernel(u_h, are_h, aim_h, bre_h, bim_h, cre_h, cim_h, ldt_h, dsk_h, x_h, wqkv_h, wo_h,
            f_h, fi_h, g_h, ones_h, o_h,
            u_v, par_v, ldt_v, dsk_v, x_v, wqkv_v, wo_v, f_v, fi_v, g_v, ones_v,
            pw, xs, kf, uf, pq_s, oa, ob, sems, osem):
    cps = []
    def cp(s, d):
        c = pltpu.make_async_copy(s, d, sems.at[len(cps)]); c.start(); cps.append(c); return c
    c_par = [cp(h, par_v.at[i]) for i, h in enumerate((are_h, aim_h, bre_h, bim_h, cre_h, cim_h))]
    c_par.append(cp(ldt_h, ldt_v))
    c_w = [cp(wqkv_h, wqkv_v), cp(x_h, x_v)]
    c_u = [cp(f_h, f_v), cp(u_h, u_v), cp(g_h, g_v)]
    c_r = [cp(ones_h, ones_v), cp(wo_h, wo_v), cp(fi_h, fi_v), cp(dsk_h, dsk_v)]

    for c in c_par: c.wait()
    dt = jnp.exp(jnp.broadcast_to(ldt_v[...].astype(f32).reshape(1, D), (N, D)).T).astype(bf16).astype(f32)
    lr, li = dt * par_v[0].astype(f32), dt * par_v[1].astype(f32)
    m = jnp.exp(lr)
    z = (m * jnp.cos(li), m * jnp.sin(li))
    p, zz = 1, {}
    while p <= 2048:
        zz[p] = z
        if p in PW:
            pw[PW[p], 0], pw[PW[p], 1] = z
        z = (z[0] * z[0] - z[1] * z[1], 2.0 * z[0] * z[1]); p *= 2
    z252 = _cmul(_cmul(_cmul(zz[4], zz[8]), _cmul(zz[16], zz[32])), _cmul(zz[64], zz[128]))
    pw[11, 0], pw[11, 1] = z252
    cb = _cmul((par_v[4].astype(f32), par_v[5].astype(f32)),
               (dt * par_v[2].astype(f32), dt * par_v[3].astype(f32)))
    pw[CI, 0], pw[CI, 1] = cb

    sub = lax.broadcasted_iota(jnp.int32, (8, 128), 0)
    lane_g = lax.broadcasted_iota(jnp.int32, (8, 128), 1) // 32
    one = (jnp.ones((8, 128), f32), jnp.zeros((8, 128), f32))

    def kgroup(g, _):
        At, Bt = [], []
        for ch in range(4):
            d = g * 4 + ch
            cache = {}
            def ld(i):
                if i not in cache:
                    cache[i] = tuple(jnp.broadcast_to(pw[i, r, pl.ds(d, 1), :], (8, 128)) for r in (0, 1))
                return cache[i]
            def selq(ps):
                out = ld(PW[ps[-1]]) if ps[-1] else one
                for q in range(len(ps) - 2, -1, -1):
                    v = ld(PW[ps[q]]) if ps[q] else one
                    out = tuple(jnp.where(sub <= q, v[r], out[r]) for r in (0, 1))
                return out
            v0 = _cmul(ld(CI), selq([None, 4, 256, 512, 1024, 2048]))
            m1 = selq([1, 1, 2, 4, 256])
            m2 = tuple(jnp.where(sub == 3, ld(11)[r], m1[r]) for r in (0, 1))
            v1 = _cmul(v0, m1); v2 = _cmul(v1, m2); v3 = _cmul(v2, m1)
            for v in (v0, v1, v2, v3):
                At.append(jnp.concatenate([v[0], -v[1]], 1))
            def bit(pV, msk):
                v = ld(PW[pV])
                return tuple(jnp.where((sub & msk) != 0, v[r], one[r]) for r in (0, 1))
            b = _cmul(_cmul(bit(8, 1), bit(16, 2)), bit(32, 4))
            for i in range(4):
                Bt.append(jnp.concatenate(b, 1))
                if i < 3:
                    b = _cmul(b, ld(PW[64]))
        A = jnp.concatenate(At, 0).astype(bf16)
        B = jnp.concatenate(Bt, 0).astype(bf16)
        o = lax.dot_general(A, B, (((1,), (1,)), ((), ())), preferred_element_type=f32)
        for ch in range(4):
            acc = None
            for c in range(4):
                t = o[ch * 32 + c * 8: ch * 32 + c * 8 + 8, :]
                s = (32 * (c - ch)) % 128
                if s: t = pltpu.roll(t, s, 1)
                acc = t if acc is None else jnp.where(lane_g == c, t, acc)
            xs[pl.ds(g * 4 + ch, 8, stride=D), :] = acc
        return 0

    for c in c_w: c.wait()
    R = 256
    def phi(t):
        t = t.astype(bf16).astype(f32)
        return jnp.where(t > 0, t + 1.0, jnp.exp(t)) + 1e-6
    kv = [jnp.zeros((128, 128), f32) for _ in range(4)]
    zs = jnp.zeros((1, D), f32)
    def step(i, carry):
        kv, zs = list(carry[0]), carry[1]
        rs = pl.ds(pl.multiple_of(i * R, R), R)
        xb = x_v[rs, :]
        mm = lambda j: jnp.dot(xb, wqkv_v[:, j * D:(j + 1) * D], preferred_element_type=f32)
        pq_s[rs, :] = phi(mm(0)).astype(bf16)
        pk = phi(mm(1)).astype(bf16)
        v = mm(2).astype(bf16)
        zs = zs + jnp.sum(pk.astype(f32), 0, keepdims=True)
        for g in range(4):
            sl = slice(g * 128, g * 128 + 128)
            kv[g] = kv[g] + lax.dot_general(pk[:, sl], v[:, sl], (((0,), (0,)), ((), ())),
                                            preferred_element_type=f32)
        for j in range(128 * R // L):
            kgroup(i * (128 * R // L) + j, 0)
        return kv, zs
    kv, zs = lax.fori_loop(0, L // R, step, (kv, zs))

    for c in c_u: c.wait()
    sg = jnp.where((sub & 1) == 0, 1.0, -1.0).astype(f32)
    sg = jnp.concatenate([jnp.tile(sg, (1, 4))] * 16, 0)
    prev = None
    for a in range(NB):
        U = jnp.dot(f_v[...], u_v[a * T:(a + 1) * T, :], preferred_element_type=f32)
        r, im = sg * U[T:], -sg * U[:T]
        if prev is not None:
            r, im = r + prev[:T], im + prev[T:]
        uf[a, 0], uf[a, 1], uf[a, 2] = r + im, im, r
        prev = U
    xq = {}
    seen = set()
    for i, (q, p_) in enumerate(_KEYS):
        if q not in xq:
            xq = {q: xs[q * D:(q + 1) * D, :].astype(bf16)}
        t = lax.dot_general(g_v[i], xq[q], (((1,), (1,)), ((), ())), preferred_element_type=f32)
        t = (t[:T], t[:T] + t[T:], t[T:] - t[:T])
        if p_ in seen:
            for e in range(3): kf[p_, e] += t[e]
        else:
            for e in range(3): kf[p_, e] = t[e]
        seen.add(p_)

    for c in c_r: c.wait()
    hm = ones_v[...].astype(f32)
    M = jnp.concatenate([
        jnp.dot((kv[g] * hm).astype(bf16), wo_v[g * 128:(g + 1) * 128, :], preferred_element_type=f32)
        for g in range(4)], 0).astype(bf16)
    zb = zs.astype(bf16).astype(f32)
    outs = []
    for a in range(NB):
        rows = slice(a * T, (a + 1) * T)
        yr, yi = [], []
        for s in range(0, T, 16):
            ac = None
            for p_ in range(a + 1):
                t = [kf[p_, e, s:s + 16, :] * uf[a - p_, e, s:s + 16, :] for e in range(3)]
                ac = t if ac is None else [v + w for v, w in zip(ac, t)]
            yr.append((ac[0] - ac[1]).astype(bf16)); yi.append((ac[0] + ac[2]).astype(bf16))
        Y = jnp.concatenate(yr + yi, 0)
        y = jnp.dot(fi_v[...], Y, preferred_element_type=f32).astype(bf16)
        ua = u_v[rows, :]
        oa[rows, :] = (y.astype(f32) + (ua.astype(f32) * dsk_v[...].astype(f32).reshape(1, D)).astype(bf16).astype(f32)).astype(bf16)
        pq = pq_s[rows, :].astype(f32)
        pz = (pq * zb).astype(bf16)
        den = jnp.concatenate([jnp.dot(pz[:, g * 128:(g + 1) * 128], ones_v[...], preferred_element_type=f32)
                               for g in range(4)], 1) + 1e-6
        ob[rows, :] = jnp.dot((pq / den).astype(bf16), M, preferred_element_type=f32).astype(bf16)
        for j, s_ in enumerate((oa, ob)):
            c = pltpu.make_async_copy(s_.at[rows, :], o_h.at[rows, pl.ds(j * D, D)], osem.at[j, a])
            c.start(); outs.append(c)
    for c in outs: c.wait()


@jax.jit
def pallas_concat_heads__ssm_conv_s4__linear_attn_block__prompt_kernel(
        A_u, A_A_re, A_A_im, A_B_re, A_B_im, A_C_re, A_C_im, A_log_dt, A_Dskip, B_x, B_wqkv, B_wo):
    V = pltpu.VMEM
    scratch = [V((L, D), bf16), V((6, D, N), bf16), V((D,), bf16), V((D,), bf16), V((L, D), bf16),
               V((D, 3 * D), bf16), V((D, D), bf16), V(_F.shape, bf16), V(_FI.shape, bf16),
               V(_G.shape, bf16), V((128, 128), bf16),
               V((13, 2, D, N), f32), V((8 * D, 128), f32), V((NB, 3, T, D), f32), V((NB, 3, T, D), f32),
               V((L, D), bf16), V((L, D), bf16), V((L, D), bf16),
               pltpu.SemaphoreType.DMA((16,)), pltpu.SemaphoreType.DMA((2, NB))]
    any_ = pl.BlockSpec(memory_space=pl.ANY)
    out = pl.pallas_call(
        _kernel, out_shape=jax.ShapeDtypeStruct((L, 2 * D), bf16),
        in_specs=[any_] * 16, out_specs=any_, scratch_shapes=scratch,
        compiler_params=pltpu.CompilerParams(vmem_limit_bytes=100 * 1024 * 1024),
    )(A_u.reshape(L, D), A_A_re, A_A_im, A_B_re, A_B_im, A_C_re, A_C_im,
      A_log_dt, A_Dskip, B_x.reshape(L, D), B_wqkv, B_wo,
      _F, _FI, _G, _ONES)
    return out.reshape(1, L, 2 * D)
```
